```python
import jax
import jax.numpy as jnp

def _softmax(x, axis=-1):
    return jax.nn.softmax(x, axis=axis)
def _gelu(x):
    return jax.nn.gelu(x, approximate=True)
def _silu(x):
    return jax.nn.silu(x)
def _sigmoid(x):
    return jax.nn.sigmoid(x)
def _layernorm(x, axis=-1, eps=1e-5):
    m = jnp.mean(x, axis=axis, keepdims=True)
    v = jnp.var(x, axis=axis, keepdims=True)
    return (x - m) / jnp.sqrt(v + eps)
def _scatter_add(tgt, idx, src, axis=0):
    return tgt.at[idx].add(src)
def _segment_sum(src, seg, n):
    return jax.ops.segment_sum(src, seg, n)
class _Rng:
    def __init__(self, key):
        self._k = key
    def _next(self):
        self._k, sub = jax.random.split(self._k)
        return sub
    def normal(self, shape):
        return jax.random.normal(self._next(), shape, dtype=jnp.bfloat16)
    def randint(self, lo, hi, shape):
        return jax.random.randint(self._next(), shape, lo, hi, dtype=jnp.int32)
    def uniform(self, shape, lo=0.0, hi=1.0):
        return jax.random.uniform(self._next(), shape, jnp.bfloat16, lo, hi)
    def permutation(self, n):
        return jax.random.permutation(self._next(), n)


kernel_name = 'parallel_sum__sliding_local_dilated__glu_gated_geglu__prompt'

def setup_inputs():
    _rng = _Rng(jax.random.key(int.from_bytes(__import__("os").urandom(4), "little")))
    _w = (lambda a: (lambda t: t.astype(jnp.bfloat16) if jnp.issubdtype(t.dtype, jnp.floating) else t)(jnp.asarray(a)))
    def _A_setup():
        B, S, D = 1, 2048, 1024
        return {
            "x": _w((lambda *s: _rng.normal(s) * 0.05)(B, S, D)),
            "wqkv": _w((lambda *s: _rng.normal(s) * 0.05)(D, 3 * D)),
            "wo": _w((lambda *s: _rng.normal(s) * 0.05)(D, D)),
        }
    _A_in = _A_setup()

    def _B_setup():
        B, S, Dm, Df = 1, 2048, 1024, 3584
        return {
            "x": _w((lambda *s: _rng.normal(s) * 0.05)(B, S, Dm)),
            "w_gate": _w((lambda *s: _rng.normal(s) * 0.05)(Dm, Df) * (Dm ** -0.5)),
            "w_up": _w((lambda *s: _rng.normal(s) * 0.05)(Dm, Df) * (Dm ** -0.5)),
            "w_down": _w((lambda *s: _rng.normal(s) * 0.05)(Df, Dm) * (Df ** -0.5)),
        }
    _B_in = _B_setup()

    return {
        "A_x": _A_in["x"],
        "A_wqkv": _A_in["wqkv"],
        "A_wo": _A_in["wo"],
        "B_x": _B_in["x"],
        "B_w_gate": _B_in["w_gate"],
        "B_w_up": _B_in["w_up"],
        "B_w_down": _B_in["w_down"],
    }

def reference(A_x, A_wqkv, A_wo, B_x, B_w_gate, B_w_up, B_w_down):
    def _A_ref(x, wqkv, wo):
        B, S, D = x.shape
        H = 32; Dh = D // H
        W, dil = 8, 2
        qkv = (lambda x, *d: x.transpose(*d))((x @ wqkv).reshape(B, S, 3, H, Dh), 2, 0, 3, 1, 4)
        q, k, v = qkv[0], qkv[1], qkv[2]
        scale = Dh ** -0.5
        pos = jnp.arange(S)
        off = jnp.arange(W) * dil
        idx = pos[:, None] - off[None, :]
        mask = idx >= 0
        idx_c = jnp.where(mask, idx, 0).reshape(-1)
        kg = k[:, :, idx_c, :].reshape(B, H, S, W, Dh)
        vg = v[:, :, idx_c, :].reshape(B, H, S, W, Dh)
        logits = jnp.einsum("bhsd,bhswd->bhsw", q, kg) * scale
        logits = jnp.where(mask[None, None, :, :], logits, -1e9)
        attn = _softmax(logits, axis=-1)
        o = jnp.einsum("bhsw,bhswd->bhsd", attn, vg)
        return (lambda x, *d: x.transpose(*d))(o, 0, 2, 1, 3).reshape(B, S, D) @ wo

    def _B_ref(x, w_gate, w_up, w_down):
        g = jnp.einsum("bsd,df->bsf", x, w_gate)
        u = jnp.einsum("bsd,df->bsf", x, w_up)
        h = _gelu(g) * u
        return jnp.einsum("bsf,fd->bsd", h, w_down)

    x = A_x
    xn = _layernorm(x, axis=-1)
    return x + _A_ref(xn, A_wqkv, A_wo) + _B_ref(xn, B_w_gate, B_w_up, B_w_down)
```

```python
import functools
import jax
import jax.numpy as jnp
import numpy as np
import jax.experimental.pallas as pl
import jax.experimental.pallas.tpu as pltpu

S, D, F = 2048, 1024, 3584
NH, DH = 32, 32
WIN, DIL = 8, 2
HALO = 16
TM = 256
HM = TM // 2
NT = S // TM
D2, F2 = D // 2, F // 2
CW = 256
NC = F2 // CW
NP = 3 * D2 // CW
NO = D2 // 128
LN_EPS = 1e-5
SCALE = DH ** -0.5
bf16, f32, i32 = jnp.bfloat16, jnp.float32, jnp.int32


def _shuffle(tiles, src1, src2):
    r = tiles[0].shape[0]
    lane = jax.lax.broadcasted_iota(i32, (r, 128), 1)
    cur = [jnp.take_along_axis(tiles[c], src1(lane, c), axis=1) for c in range(8)]
    for b in (1, 2, 4):
        msk = ((lane >> 4) & b) != 0
        cur = [jnp.where(msk, cur[(m + b) % 8], cur[m]) for m in range(8)]
    return [jnp.take_along_axis(cur[(-j) % 8], src2(lane, j), axis=1) for j in range(8)]


def _to_dmajor(tiles):
    s1 = lambda l, c: ((l >> 2) & 3) * 32 + (((l >> 4) - c) & 7) * 4 + (l & 3)
    s2 = lambda l, j: ((((l & 31) >> 2) + j) & 7) * 16 + (l & 3) * 4 + (l >> 5)
    return _shuffle(tiles, s1, s2)


def _to_hmajor(tiles):
    s1 = lambda l, j: (l & 3) * 32 + (((l >> 4) - j) & 7) * 4 + ((l >> 2) & 3)
    s2 = lambda l, c: ((((l & 31) >> 2) + c) & 7) * 16 + (l >> 5) * 4 + (l & 3)
    return _shuffle(tiles, s1, s2)


def _a_ops(a11, a12, a21, a22):
    return [(a11 + a22).astype(bf16), (a21 + a22).astype(bf16), a11.astype(bf16), a22.astype(bf16),
            (a11 + a12).astype(bf16), (a21 - a11).astype(bf16), (a12 - a22).astype(bf16)]


def _b_ops(b11, b12, b21, b22):
    b11, b12, b21, b22 = (b.astype(f32) for b in (b11, b12, b21, b22))
    return [(b11 + b22).astype(bf16), (b12 - b22).astype(bf16), (b21 - b11).astype(bf16),
            (b11 + b12).astype(bf16), (b21 + b22).astype(bf16)]


def _combine(m):
    c11 = m[0] + m[3] - m[4] + m[6]
    c12 = m[2] + m[4]
    c21 = m[1] + m[3]
    c22 = m[0] - m[1] + m[2] + m[5]
    return c11, c12, c21, c22


class _Stream:
    def __init__(self, never, tasks):
        self.never = never
        self.count = 0
        self.tasks = list(tasks)
        self.due = {}

    def _tie(self, v, token):
        w = pltpu.bitcast(v, i32)
        t = jnp.concatenate([token] * (w.shape[0] // 8), axis=0)
        t = jnp.concatenate([t] * (w.shape[1] // 128), axis=1)
        return pltpu.bitcast(jnp.where(self.never, t, w), v.dtype)

    def _run(self, after, token):
        for start, finish, fn in self.tasks:
            if start == after:
                gate = (lambda v: v) if token is None else functools.partial(self._tie, token=token)
                for v in fn(gate):
                    w = pltpu.bitcast(v, i32)
                    for r in range(0, w.shape[0], 8):
                        for c in range(0, w.shape[1], 128):
                            piece = w[r:r + 8, c:c + 128]
                            self.due[finish] = self.due[finish] | piece if finish in self.due else piece

    def dot(self, a, b):
        if self.count == 0:
            self._run(-1, None)
        if self.count in self.due:
            a = jnp.concatenate([self._tie(a[:16], self.due.pop(self.count)), a[16:]], axis=0)
        r = jnp.dot(a, b, preferred_element_type=f32)
        self._run(self.count, pltpu.bitcast(r[:8, :128], i32))
        self.count += 1
        return r


def _kernel(x_hbm, wqkv_hbm, wo_hbm, wg_hbm, wu_hbm, wd_hbm, o_hbm,
            x_v, wqkv_v, wo_v, wg_v, wu_v, wd_v,
            sqkv, so, sg, su, sd,
            xn0, aop, qkv_v, q_s, k_s, v_s, att_s, oa_s, h_s, o_v,
            sem_x, sem_qkv, sem_f, sem_wo, sem_o):

    def x_copy(t):
        rows = pl.ds(pl.multiple_of(t * TM, TM), TM)
        return pltpu.make_async_copy(x_hbm.at[rows], x_v.at[rows], sem_x.at[t])

    def qkv_copies(p):
        c0 = (p // 2) * D + (p % 2) * CW
        return [pltpu.make_async_copy(wqkv_hbm.at[:, pl.ds(c0 + h * D2, CW)], wqkv_v.at[p, h], sem_qkv.at[p])
                for h in range(2)]

    def ffn_start(c):
        for h in range(2):
            cols = pl.ds(pl.multiple_of(h * F2 + c * CW, CW), CW)
            pltpu.make_async_copy(wg_hbm.at[:, cols], wg_v.at[c, h], sem_f.at[c]).start()
            pltpu.make_async_copy(wu_hbm.at[:, cols], wu_v.at[c, h], sem_f.at[c]).start()
            pltpu.make_async_copy(wd_hbm.at[cols, :], wd_v.at[h, c], sem_f.at[c]).start()

    def ffn_wait(c):
        pltpu.make_async_copy(wg_v.at[c], wg_v.at[c], sem_f.at[c]).wait()
        pltpu.make_async_copy(wu_v.at[c], wu_v.at[c], sem_f.at[c]).wait()
        pltpu.make_async_copy(wd_v.at[:, c], wd_v.at[:, c], sem_f.at[c]).wait()

    def wo_start(c):
        for h in range(2):
            cols = pl.ds(pl.multiple_of(h * D2 + c * 128, 128), 128)
            pltpu.make_async_copy(wo_hbm.at[:, cols], wo_v.at[h, c], sem_wo.at[c]).start()

    x_copy(0).start()
    for cp in qkv_copies(0):
        cp.start()
    x_copy(1).start()
    for p in range(1, NP):
        for cp in qkv_copies(p):
            cp.start()
    x_copy(2).start()
    ffn_start(0)
    wo_start(0)

    def layernorm(rows, gate=lambda v: v):
        x = gate(x_v[rows, :]).astype(f32)
        xc = x - jnp.mean(x, axis=-1, keepdims=True)
        var = jnp.mean(xc * xc, axis=-1, keepdims=True)
        return xc * jax.lax.rsqrt(var + LN_EPS)

    def ln_ops(t, r, n, gate=lambda v: v):
        r0 = pl.multiple_of(t * TM, TM)
        top, bot = layernorm(pl.ds(r0 + r, n), gate), layernorm(pl.ds(r0 + HM + r, n), gate)
        ops = _a_ops(top[:, :D2], top[:, D2:], bot[:, :D2], bot[:, D2:])
        return ops

    x_copy(0).wait()
    for r in range(0, TM, 16):
        xn0[r:r + 16, :] = layernorm(pl.ds(r, 16)).astype(bf16)
    x_copy(1).wait()
    for r in range(0, HM, 16):
        for n, v in enumerate(ln_ops(1, r, 16)):
            aop[1, n, r:r + 16, :] = v

    def b_task(quad, dst, r, n):
        def fn(gate):
            b11, b12, b21, b22 = quad(r, n)
            ops = _b_ops(gate(b11), b12, b21, gate(b22))
            for i, v in enumerate(ops):
                dst(i, r, n, v)
            return [ops[-1][-16:, -128:]]
        return fn

    def warmup(p, carry):
        pltpu.make_async_copy(wqkv_v.at[p], wqkv_v.at[p], sem_qkv.at[p]).wait()
        quad = lambda r, n: (wqkv_v[p, 0, r:r + n], wqkv_v[p, 1, r:r + n],
                             wqkv_v[p, 0, D2 + r:D2 + r + n], wqkv_v[p, 1, D2 + r:D2 + r + n])

        def dst(i, r, n, v):
            sqkv[p, i, r:r + n, :] = v
        st = _Stream(p < 0, [(i // 2 - 1, i // 2 + 1, b_task(quad, dst, 32 * i, 32)) for i in range(16)])
        for h in range(2):
            for l in range(2):
                for r in range(0, TM, HM):
                    res = st.dot(xn0[r:r + HM, :], wqkv_v[p, h, :, l * 128:(l + 1) * 128])
                    qkv_v[p, h, HALO + r:HALO + r + HM, l * 128:(l + 1) * 128] = res.astype(bf16)
        return carry
    jax.lax.fori_loop(0, NP, warmup, 0)

    def phase1(t, carry):
        r0 = pl.multiple_of(t * TM, TM)
        c = t - 1
        co = jnp.minimum(c, NO - 1)
        nxt = (t + 1) % NT

        @pl.when(t + 2 < NT)
        def _():
            x_copy(t + 2).start()

        @pl.when(t < NC)
        def _():
            ffn_start(t)

        @pl.when(t < NO)
        def _():
            wo_start(t)

        @pl.when(nxt != 0)
        def _():
            x_copy(nxt).wait()

        def project(st, p):
            b = [sqkv[p, 0], wqkv_v[p, 0, :D2], sqkv[p, 1], sqkv[p, 2], wqkv_v[p, 1, D2:], sqkv[p, 3], sqkv[p, 4]]
            c11, c12, c21, c22 = _combine([st.dot(aop[t, n], b[n]) for n in range(7)])
            qkv_v[p, 0, pl.ds(HALO + r0, HM), :] = c11.astype(bf16)
            qkv_v[p, 1, pl.ds(HALO + r0, HM), :] = c12.astype(bf16)
            qkv_v[p, 0, pl.ds(HALO + r0 + HM, HM), :] = c21.astype(bf16)
            qkv_v[p, 1, pl.ds(HALO + r0 + HM, HM), :] = c22.astype(bf16)

        def ln_task(r):
            def fn(gate):
                ops = ln_ops(nxt, r, 16, gate)
                for n, v in enumerate(ops):
                    oa_s[n, r:r + 16, :] = v
                return [ops[0][:, -128:]]
            return fn
        st = _Stream(t < 0, [((5 * i) // 2 - 1, (5 * i) // 2 + 3, ln_task(16 * i)) for i in range(8)])
        for p in range(NP // 2):
            project(st, p)

        ffn_wait(c)

        @pl.when(c < NO)
        def _():
            pltpu.make_async_copy(wo_v.at[:, c], wo_v.at[:, c], sem_wo.at[c]).wait()

        def gu(w_v, s_v):
            def dst(i, r, n, v):
                s_v[c, i, r:r + n, :] = v
            return (lambda r, n: (w_v[c, 0, r:r + n], w_v[c, 1, r:r + n],
                                  w_v[c, 0, D2 + r:D2 + r + n], w_v[c, 1, D2 + r:D2 + r + n])), dst

        def dst_d(i, r, n, v):
            sd[i, c, r:r + n, :] = v

        def dst_o(i, r, n, v):
            so[i, co, r:r + n, :] = v
        quad_d = lambda r, n: (wd_v[0, c, r:r + n, :D2], wd_v[0, c, r:r + n, D2:],
                               wd_v[1, c, r:r + n, :D2], wd_v[1, c, r:r + n, D2:])
        quad_o = lambda r, n: (wo_v[0, co, r:r + n], wo_v[1, co, r:r + n],
                               wo_v[0, co, D2 + r:D2 + r + n], wo_v[1, co, D2 + r:D2 + r + n])
        work = [b_task(*gu(wg_v, sg), 32 * i, 32) for i in range(16)]
        work += [b_task(*gu(wu_v, su), 32 * i, 32) for i in range(16)]
        work += [b_task(quad_d, dst_d, 16 * i, 16) for i in range(16)]
        work += [b_task(quad_o, dst_o, 64 * i, 64) for i in range(8)]
        st = _Stream(t < 0, [((20 * i) // len(work) - 1, (20 * i) // len(work) + 1, fn) for i, fn in enumerate(work)])
        for p in range(NP // 2, NP):
            project(st, p)
        aop[nxt] = oa_s[...]
        return carry
    jax.lax.fori_loop(1, NT, phase1, 0)

    for p in range(NP):
        for h in range(2):
            first = qkv_v[p, h, HALO:2 * HALO, :].astype(f32)
            qkv_v[p, h, 0:HALO, :] = jnp.broadcast_to(first[0:1], (HALO, CW)).astype(bf16)

    def phase2(t, carry):
        r0 = pl.multiple_of(t * TM, TM)

        def relayout(g, dst, lo, r, n):
            def fn(gate):
                tiles = []
                for c in range(8):
                    h, s, l = c // 4, (c % 4) // 2, c % 2
                    tiles.append(pltpu.bitcast(gate(
                        qkv_v[2 * g + s, h, pl.ds(pl.multiple_of(r0 + lo + r, HALO), n), l * 128:(l + 1) * 128]), i32))
                outs = _to_dmajor(tiles)
                for j, v in enumerate(outs):
                    dst[j, r:r + n, :] = pltpu.bitcast(v, bf16).astype(f32)
                return [outs[-1][-8:]]
            return fn

        RB = 16

        def attend(rb):
            def fn(gate):
                b0 = rb * RB
                q = [gate(q_s[j, b0:b0 + RB, :]) for j in range(8)]
                logits = []
                for w in range(WIN):
                    k0 = HALO + b0 - DIL * w
                    acc = q[0] * k_s[0, k0:k0 + RB, :]
                    for j in range(1, 8):
                        acc = acc + q[j] * k_s[j, k0:k0 + RB, :]
                    acc = acc + pltpu.roll(acc, 64, 1)
                    acc = (acc + pltpu.roll(acc, 32, 1)) * SCALE
                    if b0 < DIL * w:
                        pos = r0 + b0 + jax.lax.broadcasted_iota(i32, (RB, 128), 0)
                        acc = jnp.where(pos >= DIL * w, acc, -1e9)
                    logits.append(acc)
                mx = functools.reduce(jnp.maximum, logits)
                es = [jnp.exp(l - mx) for l in logits]
                inv = 1.0 / functools.reduce(jnp.add, es)
                ps = [e * inv for e in es]
                outs = []
                for j in range(8):
                    acc = ps[0] * v_s[j, HALO + b0:HALO + b0 + RB, :]
                    for w in range(1, WIN):
                        k0 = HALO + b0 - DIL * w
                        acc = acc + ps[w] * v_s[j, k0:k0 + RB, :]
                    outs.append(acc.astype(bf16))
                    att_s[j, b0:b0 + RB, :] = outs[-1]
                return outs
            return fn

        def att_ops(r, n):
            def fn(gate):
                halves = []
                for r1 in (r, HM + r):
                    tiles = _to_hmajor([pltpu.bitcast(gate(att_s[j, r1:r1 + n, :]), i32) for j in range(8)])
                    halves.append(jnp.concatenate([pltpu.bitcast(v, bf16) for v in tiles], axis=1).astype(f32))
                top, bot = halves
                ops = _a_ops(top[:, :D2], top[:, D2:], bot[:, :D2], bot[:, D2:])
                for i, v in enumerate(ops):
                    oa_s[i, r:r + n, :] = v
                return [ops[0][-16:, -128:]]
            return fn

        tasks = []
        i = 0
        for r in range(0, TM, 64):
            for g, dst, lo in ((0, q_s, HALO), (1, k_s, 0), (2, v_s, 0)):
                n = 64 + (HALO if g and r == 0 else 0)
                tasks.append((i - 1, i + 2, relayout(g, dst, lo, r + (HALO if g and r else 0), n)))
                i += 1
        for rb in range(TM // RB):
            s0 = 13 + (9 * rb) // 2
            tasks.append((s0, s0 + 6, attend(rb)))
        for i in range(4):
            tasks.append((87 + 2 * i, 91 + 2 * i, att_ops(32 * i, 32)))
        st = _Stream(t < 0, tasks)

        for c in range(NC):
            gu = []
            for w_v, s_v in ((wg_v, sg), (wu_v, su)):
                b = [s_v[c, 0], w_v[c, 0, :D2], s_v[c, 1], s_v[c, 2], w_v[c, 1, D2:], s_v[c, 3], s_v[c, 4]]
                gu.append(_combine([st.dot(aop[t, n], b[n]) for n in range(7)]))
            h = [jax.nn.gelu(g, approximate=True) * u for g, u in zip(*gu)]
            for n, v in enumerate(_a_ops(*h)):
                h_s[n, :, c * CW:(c + 1) * CW] = v

        wide = lambda ref: jnp.concatenate([ref[i] for i in range(NO)], axis=1)
        bo = [wide(so.at[0]), wide(wo_v.at[0, :, :D2]), wide(so.at[1]), wide(so.at[2]), wide(wo_v.at[1, :, D2:]),
              wide(so.at[3]), wide(so.at[4])]
        bd = [sd[0], wd_v[0, :, :, :D2], sd[1], sd[2], wd_v[1, :, :, D2:], sd[3], sd[4]]
        m = [st.dot(oa_s[n], bo[n]) for n in range(7)]
        m = [m[n] + st.dot(h_s[n], bd[n].reshape(F2, D2)) for n in range(7)]
        c11, c12, c21, c22 = _combine(m)
        top, bot = pl.ds(r0, HM), pl.ds(r0 + HM, HM)
        o_v[top, :D2] = (c11 + x_v[top, :D2].astype(f32)).astype(bf16)
        o_v[top, D2:] = (c12 + x_v[top, D2:].astype(f32)).astype(bf16)
        o_v[bot, :D2] = (c21 + x_v[bot, :D2].astype(f32)).astype(bf16)
        o_v[bot, D2:] = (c22 + x_v[bot, D2:].astype(f32)).astype(bf16)
        pltpu.make_async_copy(o_v.at[pl.ds(r0, TM)], o_hbm.at[pl.ds(r0, TM)], sem_o).start()
        return carry
    jax.lax.fori_loop(0, NT, phase2, 0)
    pltpu.make_async_copy(o_v, o_hbm, sem_o).wait()


@jax.jit
def pallas_parallel_sum__sliding_local_dilated__glu_gated_geglu__prompt_kernel(A_x, A_wqkv, A_wo, B_x, B_w_gate, B_w_up, B_w_down):
    x = A_x.reshape(S, D)
    V = pltpu.VMEM
    DMA = pltpu.SemaphoreType.DMA
    out = pl.pallas_call(
        _kernel,
        in_specs=[pl.BlockSpec(memory_space=pl.ANY)] * 6,
        out_specs=pl.BlockSpec(memory_space=pl.ANY),
        out_shape=jax.ShapeDtypeStruct((S, D), A_x.dtype),
        scratch_shapes=[
            V((S, D), bf16), V((NP, 2, D, CW), bf16), V((2, NO, D, 128), bf16),
            V((NC, 2, D, CW), bf16), V((NC, 2, D, CW), bf16), V((2, NC, CW, D), bf16),
            V((NP, 5, D2, CW), bf16), V((5, NO, D2, 128), bf16),
            V((NC, 5, D2, CW), bf16), V((NC, 5, D2, CW), bf16), V((5, NC, CW, D2), bf16),
            V((TM, D), bf16), V((NT, 7, HM, D2), bf16), V((NP, 2, S + HALO, CW), bf16),
            V((8, TM, 128), f32), V((8, TM + HALO, 128), f32), V((8, TM + HALO, 128), f32),
            V((8, TM, 128), bf16), V((7, HM, D2), bf16),
            V((7, HM, F2), bf16), V((S, D), bf16),
            DMA((NT,)), DMA((NP,)), DMA((NC,)), DMA((NO,)), DMA(()),
        ],
        compiler_params=pltpu.CompilerParams(vmem_limit_bytes=120 * 1024 * 1024),
    )(x, A_wqkv, A_wo, B_w_gate, B_w_up, B_w_down)
    return out.reshape(A_x.shape)
```

```python
import functools
import jax
import jax.numpy as jnp
import numpy as np
import jax.experimental.pallas as pl
import jax.experimental.pallas.tpu as pltpu

S, D, F = 2048, 1024, 3584
NH, DH = 32, 32
WIN, DIL = 8, 2
HALO = 16
L = 128
TM = 256
HM = TM // 2
QM = TM // 4
NT = S // TM
D2, F2 = D // 2, F // 2
CW = 256
DL = D2 // L
NC = F2 // CW
NP = 3 * D2 // CW
LN_EPS = 1e-5
SCALE = DH ** -0.5
bf16, f32, i32 = jnp.bfloat16, jnp.float32, jnp.int32


def _pack(v):
    return pltpu.bitcast(v.astype(bf16), i32)


def _bf(words):
    return pltpu.bitcast(words, bf16)


def _pack_groups(v):
    lo, hi = ([v[r:r + 8] for r in range(k, v.shape[0], 16)] for k in (0, 8))
    return pltpu.pack_elementwise([jnp.concatenate(lo, axis=0), jnp.concatenate(hi, axis=0)], packed_dtype=bf16)


def _unpack_group(words):
    return jnp.concatenate(
        [pltpu.unpack_elementwise(words, index=k, packed_dtype=bf16, unpacked_dtype=f32) for k in range(2)], axis=0)


def _group(shape):
    return jax.lax.broadcasted_iota(i32, shape, 1) >> 2


def _exchange(tiles, b):
    take = (_group(tiles[0].shape) & b) != 0
    n = len(tiles) // 2
    return ([jnp.where(take, hi, lo) for lo, hi in zip(tiles[:n], tiles[n:])]
            + [jnp.where(take, lo, hi) for lo, hi in zip(tiles[:n], tiles[n:])])


def _butterfly(tiles, b):
    if len(tiles) == 1:
        return tiles
    tiles = _exchange(tiles, b)
    n = len(tiles) // 2
    return _butterfly(tiles[:n], b // 2) + _butterfly(tiles[n:], b // 2)


def _spread(tile, m):
    lane = jax.lax.broadcasted_iota(i32, tile.shape, 1)
    return jnp.take_along_axis(tile, (lane & 3) * 32 + ((lane >> 2) ^ m), axis=1)


def _unspread(tile, m):
    lane = jax.lax.broadcasted_iota(i32, tile.shape, 1)
    return jnp.take_along_axis(tile, ((lane & 31) ^ m) * 4 + (lane >> 5), axis=1)


def _flip(tile, d):
    lane = jax.lax.broadcasted_iota(i32, tile.shape, 1)
    return jnp.take_along_axis(tile, lane ^ (4 * d), axis=1) if d else tile


def _a_ops(a11, a12, a21, a22):
    return [a11 + a22, a21 + a22, a11, a22, a11 + a12, a21 - a11, a12 - a22]


def _b_ops(b11, b12, b21, b22):
    b11, b12, b21, b22 = (b.astype(f32) for b in (b11, b12, b21, b22))
    return [_pack(v) for v in (b11 + b22, b12 - b22, b21 - b11, b11 + b12, b21 + b22)]


def _combine(m):
    c11 = m[0] + m[3] - m[4] + m[6]
    c12 = m[2] + m[4]
    c21 = m[1] + m[3]
    c22 = m[0] - m[1] + m[2] + m[5]
    return c11, c12, c21, c22


def _half(r, n):
    return slice(r // 2, (r + n) // 2)


class _Stream:
    def __init__(self, never, tasks):
        self.never = never
        self.count = 0
        self.tasks = list(tasks)
        self.due = {}

    def _tie(self, v, token):
        w = pltpu.bitcast(v, i32)
        t = jnp.concatenate([token] * (w.shape[0] // 8), axis=0)
        t = jnp.concatenate([t] * (w.shape[1] // L), axis=1)
        return pltpu.bitcast(jnp.where(self.never, t, w), v.dtype)

    def _run(self, result):
        for start, finish, fn in self.tasks:
            if result is None and start < 0:
                gate = lambda v: v
            elif result is not None and self.count <= start < self.count + 1:
                rows, cols = result.shape[0] // 8, result.shape[1] // L
                at = int((start - self.count) * rows * cols)
                r, c = at % rows * 8, at // rows * L
                gate = functools.partial(self._tie, token=pltpu.bitcast(result[r:r + 8, c:c + L], i32))
            else:
                continue
            for v in fn(gate):
                w = pltpu.bitcast(v, i32)
                for r in range(0, w.shape[0], 8):
                    for c in range(0, w.shape[1], L):
                        piece = w[r:r + 8, c:c + L]
                        self.due[finish] = self.due[finish] | piece if finish in self.due else piece

    def dot(self, a, b):
        if self.count == 0:
            self._run(None)
        if self.count in self.due:
            a = jnp.concatenate([self._tie(a[:16], self.due.pop(self.count)), a[16:]], axis=0)
        r = jnp.dot(a, b, preferred_element_type=f32)
        self._run(r)
        self.count += 1
        return r


def _kernel(x_hbm, wqkv_hbm, wo_hbm, wg_hbm, wu_hbm, wd_hbm, o_hbm,
            x_v, wqkv_v, wo_v, wg_v, wu_v, wd_v,
            sqkv, so, sg, su, sd,
            xn0, aop, qkv_v, q_s, k_s, v_s, att_s, oa_s, a_s, h_s, o_v,
            sem_x, sem_qkv, sem_f, sem_wo, sem_o):

    def x_copy(t):
        rows = pl.ds(pl.multiple_of(t * TM, TM), TM)
        return pltpu.make_async_copy(x_hbm.at[rows], x_v.at[rows], sem_x.at[t])

    def qkv_start(p):
        c0 = (p // 2) * D + (p % 2) * CW
        for h in range(2):
            pltpu.make_async_copy(wqkv_hbm.at[:, pl.ds(c0 + h * D2, CW)], wqkv_v.at[p, h], sem_qkv.at[p]).start()

    def ffn_start(c):
        for h in range(2):
            cols = pl.ds(pl.multiple_of(h * F2 + c * CW, CW), CW)
            pltpu.make_async_copy(wg_hbm.at[:, cols], wg_v.at[c, h], sem_f.at[c]).start()
            pltpu.make_async_copy(wu_hbm.at[:, cols], wu_v.at[c, h], sem_f.at[c]).start()
            pltpu.make_async_copy(wd_hbm.at[cols, :], wd_v.at[h, c], sem_f.at[c]).start()

    def ffn_wait(c):
        pltpu.make_async_copy(wg_v.at[c], wg_v.at[c], sem_f.at[c]).wait()
        pltpu.make_async_copy(wu_v.at[c], wu_v.at[c], sem_f.at[c]).wait()
        pltpu.make_async_copy(wd_v.at[:, c], wd_v.at[:, c], sem_f.at[c]).wait()

    def wo_start(c):
        for h in range(2):
            cols = pl.ds(pl.multiple_of(h * D2 + c * L, L), L)
            pltpu.make_async_copy(wo_hbm.at[:, cols], wo_v.at[h, c], sem_wo.at[c]).start()

    def layernorm(rows, gate=lambda v: v):
        x = gate(x_v[rows, :].astype(f32))
        xc = x - jnp.mean(x, axis=-1, keepdims=True)
        var = jnp.mean(xc * xc, axis=-1, keepdims=True)
        return xc * jax.lax.rsqrt(var + LN_EPS)

    def ln_ops(t, r, n, gate=lambda v: v):
        r0 = pl.multiple_of(t * TM, TM)
        top, bot = layernorm(pl.ds(r0 + r, n), gate), layernorm(pl.ds(r0 + HM + r, n), gate)
        return [_pack(v) for v in _a_ops(top[:, :D2], top[:, D2:], bot[:, :D2], bot[:, D2:])]

    x_copy(0).start()
    qkv_start(0)
    x_copy(0).wait()
    x_copy(1).start()
    qkv_start(1)
    for r in range(0, TM, 16):
        xn0[_half(r, 16), :] = _pack(layernorm(pl.ds(r, 16)))
    x_copy(1).wait()
    for p in range(2, NP):
        qkv_start(p)
    for r in range(0, HM, 16):
        for n, v in enumerate(ln_ops(1, r, 16)):
            aop[1, n, _half(r, 16), :] = v
            oa_s[n, _half(r, 16), :] = v

    def b_task(quad, dst, r, n):
        def fn(gate):
            b11, b12, b21, b22 = quad(r, n)
            ops = _b_ops(gate(b11.astype(f32)), b12, b21, b22)
            for i, v in enumerate(ops):
                dst(i)[_half(r, n), :] = v
            return [ops[-1][-8:, -L:]]
        return fn

    def column_quad(w):
        return lambda r, n: (w[0, r:r + n], w[1, r:r + n], w[0, D2 + r:D2 + r + n], w[1, D2 + r:D2 + r + n])

    def right_ops(s, b11, b22):
        return [_bf(s[0]), b11, _bf(s[1]), _bf(s[2]), b22, _bf(s[3]), _bf(s[4])]

    def warmup(p, carry):
        pltpu.make_async_copy(wqkv_v.at[p], wqkv_v.at[p], sem_qkv.at[p]).wait()

        @pl.when(p == 1)
        def _():
            x_copy(2).start()

        @pl.when(p == 2)
        def _():
            ffn_start(0)
            wo_start(0)

        st = _Stream(p < 0, [(i / 2 - 0.5, i // 2 + 2,
                              b_task(column_quad(wqkv_v.at[p]), lambda i: sqkv.at[p, i], 32 * i, 32))
                             for i in range(16)])
        for h in range(2):
            for l in range(0, CW, L):
                for r in range(0, TM, HM):
                    res = st.dot(_bf(xn0[_half(r, HM), :]), wqkv_v[p, h, :, l:l + L])
                    qkv_v[p, h, _half(HALO + r, HM), l:l + L] = _pack_groups(res)
        return carry
    jax.lax.fori_loop(0, NP, warmup, 0)

    def phase1(t, carry):
        r0 = pl.multiple_of(t * HM, HM)
        c = t - 1
        co = jnp.minimum(c, DL - 1)
        nxt = (t + 1) % NT

        @pl.when(nxt != 0)
        def _():
            x_copy(nxt).wait()

        @pl.when(t + 2 < NT)
        def _():
            x_copy(t + 2).start()

        def project(st, p):
            b = right_ops(sqkv.at[p], wqkv_v[p, 0, :D2], wqkv_v[p, 1, D2:])
            m = []
            for n in range(7):
                m.append(st.dot(_bf(oa_s[n]), b[n]))
                if p == NP - 1:
                    oa_s[n] = aop[nxt, n]
            c11, c12, c21, c22 = _combine(m)
            top, bot = pl.ds(r0 + HALO // 2, HM // 2), pl.ds(r0 + (HALO + HM) // 2, HM // 2)
            qkv_v[p, 0, top, :] = _pack_groups(c11)
            qkv_v[p, 1, top, :] = _pack_groups(c12)
            qkv_v[p, 0, bot, :] = _pack_groups(c21)
            qkv_v[p, 1, bot, :] = _pack_groups(c22)

        def ln_task(r):
            def fn(gate):
                ops = ln_ops(nxt, r, 16, gate)
                for n, v in enumerate(ops):
                    aop[nxt, n, _half(r, 16), :] = v
                return [ops[0][:, -L:]]
            return fn
        st = _Stream(t < 0, [(2.4 * i - 0.5, int(2.4 * i) + 4, ln_task(16 * i)) for i in range(8)])
        for p in range(NP // 2):
            project(st, p)

        ffn_wait(c)

        @pl.when(c < DL)
        def _():
            pltpu.make_async_copy(wo_v.at[:, c], wo_v.at[:, c], sem_wo.at[c]).wait()

        @pl.when(t < NC)
        def _():
            ffn_start(t)

        @pl.when(t < DL)
        def _():
            wo_start(t)

        quad_d = lambda r, n: (wd_v[0, c, r:r + n, :D2], wd_v[0, c, r:r + n, D2:],
                               wd_v[1, c, r:r + n, :D2], wd_v[1, c, r:r + n, D2:])
        work = [b_task(column_quad(wg_v.at[c]), lambda i: sg.at[c, i], 32 * i, 32) for i in range(16)]
        work += [b_task(column_quad(wu_v.at[c]), lambda i: su.at[c, i], 32 * i, 32) for i in range(16)]
        work += [b_task(quad_d, lambda i: sd.at[i, c], 16 * i, 16) for i in range(16)]
        work += [b_task(column_quad(wo_v.at[:, co]), lambda i: so.at[i, co], 64 * i, 64) for i in range(8)]
        step = 19.5 / len(work)
        st = _Stream(t < 0, [(step * i - 0.5, int(step * i) + 2, fn) for i, fn in enumerate(work)])
        for p in range(NP // 2, NP):
            project(st, p)
        return carry
    jax.lax.fori_loop(1, NT, phase1, 0)

    for p in range(NP):
        for h in range(2):
            first = _unpack_group(qkv_v[p, h, _half(HALO, HALO), :])
            qkv_v[p, h, _half(0, HALO), :] = _pack_groups(jnp.broadcast_to(first[0:1], (HALO, CW)))

    def phase2(t, carry):
        r0 = pl.multiple_of(t * TM, TM)
        held = {}

        def gather_heads(g, i, lo, s):
            def fn(gate):
                rows = pl.ds(pl.multiple_of(t * HM + (lo + s * QM + 16 * i) // 2, 8), 8)
                tiles = [_spread(gate(qkv_v[2 * g + (c % 4) // 2, c // 4, rows, (c % 2) * L:(c % 2 + 1) * L]), 8 * s + c)
                         for c in range(8)]
                held[g, i, s] = _butterfly(tiles, 4)
                return [held[g, i, s][-1]]
            return fn

        def gather_blocks(g, i, dst, c0):
            def fn(gate):
                for c in range(c0, c0 + 2):
                    tiles = _butterfly([gate(held[g, i, s][c]) if s == 0 else held[g, i, s][c] for s in range(4)], 16)
                    for k, v in enumerate(tiles):
                        out = _flip(v, 8 * k + c)
                        dst[8 * k + c, 16 * i:16 * i + 16, :] = _unpack_group(out)
                return [out]
            return fn

        def relayout(g, dst, i, lo):
            return [gather_heads(g, i, lo, s) for s in range(4)] + [gather_blocks(g, i, dst, c) for c in range(0, 8, 2)]

        def scores(i, d0, dn):
            def fn(gate):
                b0 = 16 * i
                logits = held.setdefault(("logits", i), [None] * WIN)
                for d in range(d0, d0 + dn):
                    q = gate(q_s[d, b0:b0 + 16, :])
                    for w in range(WIN):
                        k0 = HALO + b0 - DIL * w
                        term = q * k_s[d, k0:k0 + 16, :]
                        logits[w] = term if d == 0 else logits[w] + term
                return [logits[-1][-8:]]
            return fn

        def softmax(i):
            def fn(gate):
                logits = [l * SCALE for l in held["logits", i]]
                if i == 0:
                    pos = (r0 + QM * (jax.lax.broadcasted_iota(i32, (16, L), 1) >> 5)
                           + jax.lax.broadcasted_iota(i32, (16, L), 0))
                    logits = [jnp.where(pos >= DIL * w, l, -1e9) if w else l for w, l in enumerate(logits)]
                mx = functools.reduce(jnp.maximum, logits)
                es = [jnp.exp(l - mx) for l in logits]
                inv = 1.0 / functools.reduce(jnp.add, es)
                held["weights", i] = [e * inv for e in es]
                return [inv]
            return fn

        def values(i, d0, dn):
            def fn(gate):
                b0 = 16 * i
                ps = list(held["weights", i])
                ps[0] = gate(ps[0])
                for d in range(d0, d0 + dn):
                    acc = ps[0] * v_s[d, HALO + b0:HALO + b0 + 16, :]
                    for w in range(1, WIN):
                        k0 = HALO + b0 - DIL * w
                        acc = acc + ps[w] * v_s[d, k0:k0 + 16, :]
                    out = _pack_groups(acc)
                    att_s[d, _half(b0, 16), :] = out
                return [out]
            return fn

        def scatter_blocks(i, c0):
            def fn(gate):
                for c in range(c0, c0 + 2):
                    tiles = [_flip(gate(att_s[8 * k + c, _half(16 * i, 16), :]), 8 * k + c) for k in range(4)]
                    held["out", i, c] = _butterfly(tiles, 16)
                return [held["out", i, c][-1]]
            return fn

        def scatter_heads(i, s):
            def fn(gate):
                rows = []
                for s1 in (s, s + 2):
                    tiles = [held["out", i, c][s1] for c in range(8)]
                    tiles = _butterfly([gate(tiles[0])] + tiles[1:], 4)
                    rows.append([_unpack_group(_unspread(v, 8 * s1 + c)) for c, v in enumerate(tiles)])
                for c in range(0, 4, 2):
                    part = lambda k, c1: jnp.concatenate(rows[k][c1:c1 + 2], axis=1)
                    ops = _a_ops(part(0, c), part(0, c + 4), part(1, c), part(1, c + 4))
                    for n, v in enumerate(ops):
                        a_s[n, s * QM + 16 * i:s * QM + 16 * i + 16, c * L:(c + 2) * L] = v.astype(bf16)
                return [ops[0][-8:, -L:]]
            return fn

        tasks = []
        at = -0.2

        def place(fns, span, slack=4):
            nonlocal at
            for fn in fns:
                tasks.append((at, int(at + span) + slack, fn))
                at += span

        for i in range(4):
            place(relayout(0, q_s, i, HALO), 0.2)
            if i == 0:
                place(relayout(1, k_s, 0, 0), 0.2)
            place(relayout(1, k_s, i + 1, 0), 0.2)
            place([scores(i, d, 4) for d in range(0, DH, 4)], 0.9)
            place([softmax(i)], 0.3)
            if i == 0:
                place(relayout(2, v_s, 0, 0), 0.2)
            place(relayout(2, v_s, i + 1, 0), 0.2)
            place([values(i, d, 4) for d in range(0, DH, 4)], 0.9)
            place([scatter_blocks(i, c) for c in range(0, 8, 2)], 0.2)
            place([scatter_heads(i, s) for s in range(2)], 0.8)
        assert at < 14 * NC - 1, at
        st = _Stream(t < 0, tasks)

        for c in range(NC):
            gu = []
            for w_v, s_v in ((wg_v, sg), (wu_v, su)):
                b = right_ops(s_v.at[c], w_v[c, 0, :D2], w_v[c, 1, D2:])
                gu.append(_combine([st.dot(_bf(aop[t, n]), b[n]) for n in range(7)]))
            h = [jax.nn.gelu(g, approximate=True) * u for g, u in zip(*gu)]
            for n, v in enumerate(_a_ops(*h)):
                h_s[n, :, c * CW:(c + 1) * CW] = v.astype(bf16)

        wide = lambda ref: jnp.concatenate([ref[i] for i in range(DL)], axis=1)
        bo = right_ops([wide(so.at[i]) for i in range(5)], wide(wo_v.at[0, :, :D2]), wide(wo_v.at[1, :, D2:]))
        bd = right_ops([sd[i].reshape(F2 // 2, D2) for i in range(5)],
                       wd_v[0, :, :, :D2].reshape(F2, D2), wd_v[1, :, :, D2:].reshape(F2, D2))
        m = [st.dot(a_s[n], bo[n]) for n in range(7)]
        m = [m[n] + st.dot(h_s[n], bd[n]) for n in range(7)]
        c11, c12, c21, c22 = _combine(m)
        top, bot = pl.ds(r0, HM), pl.ds(r0 + HM, HM)
        o_v[top, :D2] = (c11 + x_v[top, :D2].astype(f32)).astype(bf16)
        o_v[top, D2:] = (c12 + x_v[top, D2:].astype(f32)).astype(bf16)
        o_v[bot, :D2] = (c21 + x_v[bot, :D2].astype(f32)).astype(bf16)
        o_v[bot, D2:] = (c22 + x_v[bot, D2:].astype(f32)).astype(bf16)
        pltpu.make_async_copy(o_v.at[pl.ds(r0, TM)], o_hbm.at[pl.ds(r0, TM)], sem_o).start()
        return carry
    jax.lax.fori_loop(0, NT, phase2, 0)
    pltpu.make_async_copy(o_v, o_hbm, sem_o).wait()


@jax.jit
def pallas_parallel_sum__sliding_local_dilated__glu_gated_geglu__prompt_kernel(A_x, A_wqkv, A_wo, B_x, B_w_gate, B_w_up, B_w_down):
    x = A_x.reshape(S, D)
    V = pltpu.VMEM
    DMA = pltpu.SemaphoreType.DMA
    out = pl.pallas_call(
        _kernel,
        in_specs=[pl.BlockSpec(memory_space=pl.ANY)] * 6,
        out_specs=pl.BlockSpec(memory_space=pl.ANY),
        out_shape=jax.ShapeDtypeStruct((S, D), A_x.dtype),
        scratch_shapes=[
            V((S, D), bf16), V((NP, 2, D, CW), bf16), V((2, DL, D, L), bf16),
            V((NC, 2, D, CW), bf16), V((NC, 2, D, CW), bf16), V((2, NC, CW, D), bf16),
            V((NP, 5, D2 // 2, CW), i32), V((5, DL, D2 // 2, L), i32),
            V((NC, 5, D2 // 2, CW), i32), V((NC, 5, D2 // 2, CW), i32), V((5, NC, CW // 2, D2), i32),
            V((TM // 2, D), i32), V((NT, 7, HM // 2, D2), i32), V((NP, 2, (S + HALO) // 2, CW), i32),
            V((DH, QM, L), f32), V((DH, QM + HALO, L), f32), V((DH, QM + HALO, L), f32),
            V((DH, QM // 2, L), i32), V((7, HM // 2, D2), i32),
            V((7, HM, D2), bf16), V((7, HM, F2), bf16), V((S, D), bf16),
            DMA((NT,)), DMA((NP,)), DMA((NC,)), DMA((DL,)), DMA(()),
        ],
        compiler_params=pltpu.CompilerParams(vmem_limit_bytes=120 * 1024 * 1024),
    )(x, A_wqkv, A_wo, B_w_gate, B_w_up, B_w_down)
    return out.reshape(A_x.shape)
```

```python
import functools
import jax
import jax.numpy as jnp
import numpy as np
import jax.experimental.pallas as pl
import jax.experimental.pallas.tpu as pltpu

S, D, F = 2048, 1024, 3584
NH, DH = 32, 32
WIN, DIL = 8, 2
HALO = 16
L = 128
TM = 256
HM = TM // 2
QM = TM // 4
NT = S // TM
D2, F2 = D // 2, F // 2
CW = 256
DL = D2 // L
NC = F2 // CW
NP = 3 * D2 // CW
NQ = 2 * NC + D2 // CW
RW = 128
NR = F2 // RW
LN_EPS = 1e-5
SCALE = DH ** -0.5
bf16, f32, i32 = jnp.bfloat16, jnp.float32, jnp.int32


def _pack(v):
    return pltpu.bitcast(v.astype(bf16), i32)


def _bf(words):
    return pltpu.bitcast(words, bf16)


def _pack_groups(v):
    lo, hi = ([v[r:r + 8] for r in range(k, v.shape[0], 16)] for k in (0, 8))
    return pltpu.pack_elementwise([jnp.concatenate(lo, axis=0), jnp.concatenate(hi, axis=0)], packed_dtype=bf16)


def _unpack_group(words):
    return jnp.concatenate(
        [pltpu.unpack_elementwise(words, index=k, packed_dtype=bf16, unpacked_dtype=f32) for k in range(2)], axis=0)


def _group(shape):
    return jax.lax.broadcasted_iota(i32, shape, 1) >> 2


def _exchange(tiles, b):
    take = (_group(tiles[0].shape) & b) != 0
    n = len(tiles) // 2
    return ([jnp.where(take, hi, lo) for lo, hi in zip(tiles[:n], tiles[n:])]
            + [jnp.where(take, lo, hi) for lo, hi in zip(tiles[:n], tiles[n:])])


def _butterfly(tiles, b):
    if len(tiles) == 1:
        return tiles
    tiles = _exchange(tiles, b)
    n = len(tiles) // 2
    return _butterfly(tiles[:n], b // 2) + _butterfly(tiles[n:], b // 2)


def _spread(tile, m):
    lane = jax.lax.broadcasted_iota(i32, tile.shape, 1)
    return jnp.take_along_axis(tile, (lane & 3) * 32 + ((lane >> 2) ^ m), axis=1)


def _unspread(tile, m):
    lane = jax.lax.broadcasted_iota(i32, tile.shape, 1)
    return jnp.take_along_axis(tile, ((lane & 31) ^ m) * 4 + (lane >> 5), axis=1)


def _flip(tile, d):
    lane = jax.lax.broadcasted_iota(i32, tile.shape, 1)
    return jnp.take_along_axis(tile, lane ^ (4 * d), axis=1) if d else tile


def _a_ops(a11, a12, a21, a22):
    return [a11 + a22, a21 + a22, a11, a22, a11 + a12, a21 - a11, a12 - a22]


def _b_ops(b11, b12, b21, b22):
    b11, b12, b21, b22 = (b.astype(f32) for b in (b11, b12, b21, b22))
    return [_pack(v) for v in (b11 + b22, b12 - b22, b21 - b11, b11 + b12, b21 + b22)]


def _combine(m):
    c11 = m[0] + m[3] - m[4] + m[6]
    c12 = m[2] + m[4]
    c21 = m[1] + m[3]
    c22 = m[0] - m[1] + m[2] + m[5]
    return c11, c12, c21, c22


def _half(r, n):
    return slice(r // 2, (r + n) // 2)


class _Stream:
    def __init__(self, never, tasks):
        self.never = never
        self.count = 0
        self.tasks = list(tasks)
        self.due = {}

    def _tie(self, v, token):
        w = pltpu.bitcast(v, i32)
        t = jnp.concatenate([token] * (w.shape[0] // 8), axis=0)
        t = jnp.concatenate([t] * (w.shape[1] // L), axis=1)
        return pltpu.bitcast(jnp.where(self.never, t, w), v.dtype)

    def after(self, v, result):
        return self._tie(v, pltpu.bitcast(result[:8, :L], i32))

    def _run(self, result):
        for start, finish, fn in self.tasks:
            if result is None and start < 0:
                gate = lambda v: v
            elif result is not None and self.count <= start < self.count + 1:
                rows, cols = result.shape[0] // 8, result.shape[1] // L
                at = int((start - self.count) * rows * cols)
                r, c = at % rows * 8, at // rows * L
                gate = functools.partial(self._tie, token=pltpu.bitcast(result[r:r + 8, c:c + L], i32))
            else:
                continue
            for v in fn(gate):
                w = pltpu.bitcast(v, i32)
                for r in range(0, w.shape[0], 8):
                    for c in range(0, w.shape[1], L):
                        piece = w[r:r + 8, c:c + L]
                        self.due[finish] = self.due[finish] | piece if finish in self.due else piece

    def dot(self, a, b):
        if self.count == 0:
            self._run(None)
        if self.count in self.due:
            a = jnp.concatenate([self._tie(a[:16], self.due.pop(self.count)), a[16:]], axis=0)
        r = jnp.dot(a, b, preferred_element_type=f32)
        self._run(r)
        self.count += 1
        return r


def _kernel(x_hbm, wqkv_hbm, wo_hbm, wg_hbm, wu_hbm, wd_hbm, o_hbm,
            x_v, wqkv_v, wc_v, wd_v, sqkv, sc, sd,
            aop, qkv_v, q_s, k_s, v_s, att_s, cur_s, nxt_s, a_s, h_s, o_v,
            sem_x, sem_qkv, sem_c, sem_d, sem_o):

    def x_copy(t):
        rows = pl.ds(pl.multiple_of(t * TM, TM), TM)
        return pltpu.make_async_copy(x_hbm.at[rows], x_v.at[rows], sem_x.at[t])

    def qkv_start(p):
        c0 = (p // 2) * D + (p % 2) * CW
        for h in range(2):
            pltpu.make_async_copy(wqkv_hbm.at[:, pl.ds(c0 + h * D2, CW)], wqkv_v.at[p, h], sem_qkv.at[p]).start()

    def column_start(q):
        w_hbm, c = ((wg_hbm, q), (wu_hbm, q - NC), (wo_hbm, q - 2 * NC))[q // NC]
        for h in range(2):
            cols = pl.ds(h * (w_hbm.shape[1] // 2) + c * CW, CW)
            pltpu.make_async_copy(w_hbm.at[:, cols], wc_v.at[q, h], sem_c.at[q]).start()

    def row_start(e):
        for h in range(2):
            pltpu.make_async_copy(wd_hbm.at[pl.ds(h * F2 + e * RW, RW)], wd_v.at[h, e], sem_d.at[e]).start()

    def layernorm(r0, n, gate):
        x = gate(x_v[pl.ds(pl.multiple_of(r0, 16), n), :].astype(f32))
        xc = x - jnp.mean(x, axis=-1, keepdims=True)
        var = jnp.mean(xc * xc, axis=-1, keepdims=True)
        return xc * jax.lax.rsqrt(var + LN_EPS)

    def ln_task(t, r, dst):
        def fn(gate):
            top, bot = layernorm(t * TM + r, 16, gate), layernorm(t * TM + HM + r, 16, gate)
            ops = [_pack(v) for v in _a_ops(top[:, :D2], top[:, D2:], bot[:, :D2], bot[:, D2:])]
            for n, v in enumerate(ops):
                dst[n, pl.ds(pl.multiple_of(r // 2, 8), 8), :] = v
            return [ops[0][:, -L:]]
        return fn

    def b_task(quad, dst, r, n):
        def fn(gate):
            b11, b12, b21, b22 = quad(r, n)
            ops = _b_ops(gate(b11.astype(f32)), b12, b21, b22)
            for i, v in enumerate(ops):
                dst(i)[_half(r, n), :] = v
            return [ops[-1][-8:, -L:]]
        return fn

    def column_tasks(w, s, n):
        quad = lambda r, n: (w[0, r:r + n], w[1, r:r + n], w[0, D2 + r:D2 + r + n], w[1, D2 + r:D2 + r + n])
        return [b_task(quad, lambda i: s.at[i], r, n) for r in range(0, D2, n)]

    def row_tasks(e, n):
        quad = lambda r, n: (wd_v[0, e, r:r + n, :D2], wd_v[0, e, r:r + n, D2:],
                             wd_v[1, e, r:r + n, :D2], wd_v[1, e, r:r + n, D2:])
        return [b_task(quad, lambda i: sd.at[i, e], r, n) for r in range(0, RW, n)]

    def right_op(n, sums, b11, b22):
        return b11() if n == 1 else b22() if n == 4 else _bf(sums((0, None, 1, 2, None, 3, 4)[n]))

    def column_op(n, w, s):
        return right_op(n, lambda i: s[i], lambda: w[0, :D2], lambda: w[1, D2:])

    def store_qkv(p, r0, blocks):
        c11, c12, c21, c22 = blocks
        top, bot = pl.ds(r0 + HALO // 2, HM // 2), pl.ds(r0 + (HALO + HM) // 2, HM // 2)
        qkv_v[p, 0, bot, :] = _pack_groups(c21)
        qkv_v[p, 1, top, :] = _pack_groups(c12)
        qkv_v[p, 1, bot, :] = _pack_groups(c22)
        qkv_v[p, 0, top, :] = _pack_groups(c11)

    x_copy(0).start()
    x_copy(1).start()
    qkv_start(0)
    x_copy(0).wait()
    x_copy(2).start()
    qkv_start(1)
    for r in range(0, HM, 16):
        ln_task(0, r, aop.at[0])(lambda v: v)
    x_copy(1).wait()
    for p in range(2, NP):
        qkv_start(p)
    for r in range(0, HM, 16):
        ln_task(1, r, aop.at[1])(lambda v: v)

    def warmup(p, carry):
        pltpu.make_async_copy(wqkv_v.at[p], wqkv_v.at[p], sem_qkv.at[p]).wait()

        @pl.when(p == 1)
        def _():
            x_copy(2).wait()

        for j in range(NP):
            @pl.when(p == j)
            def _():
                for q in range(3 * j, min(3 * j + 3, NQ)):
                    column_start(q)
                for e in range(3 * j, min(3 * j + 3, NR)):
                    row_start(e)
                if j + 3 < NT:
                    x_copy(j + 3).start()

        src, r0 = jnp.where(p == 0, 1, 2), jnp.clip(p - 1, 0, 3) * 32
        tasks = [(i / 8 - 1 / 8, 2, fn) for i, fn in enumerate(column_tasks(wqkv_v.at[p], sqkv.at[p], 32))]
        tasks += [(2.5 + 2 * i, 5 + i, ln_task(src, r0 + 16 * i, cur_s)) for i in range(2)]
        st = _Stream(p < 0, tasks)
        m = [None] * 7
        for n in (1, 4, 0, 2, 3, 5, 6):
            a = jnp.concatenate([aop[0, n], aop[1, n]], axis=0)
            m[n] = st.dot(_bf(a), column_op(n, wqkv_v.at[p], sqkv.at[p]))
        for t in range(2):
            blocks = _combine([v[t * HM:(t + 1) * HM] for v in m])
            store_qkv(p, t * HM, blocks)
            if t == 0:
                for h in range(2):
                    qkv_v[p, h, :HALO // 2, :] = _pack_groups(jnp.broadcast_to(blocks[h][0:1], (HALO, CW)))
        return carry
    jax.lax.fori_loop(0, NP, warmup, 0)

    def phase1(j, carry):
        t = j + 2
        for i in range(3):
            q = 3 * j + i

            @pl.when(q < NQ)
            def _():
                pltpu.make_async_copy(wc_v.at[q], wc_v.at[q], sem_c.at[q]).wait()

            @pl.when(q < NR)
            def _():
                pltpu.make_async_copy(wd_v.at[:, q], wd_v.at[:, q], sem_d.at[q]).wait()

        @pl.when(t + 1 < NT)
        def _():
            x_copy(t + 1).wait()

        work = []
        for i in range(3):
            q, e = jnp.minimum(3 * j + i, NQ - 1), jnp.minimum(3 * j + i, NR - 1)
            work += column_tasks(wc_v.at[q], sc.at[q], 32) + row_tasks(e, 16)
        tasks, at = [], -0.3
        for i in range(8):
            tasks.append((at, int(at) + 5, ln_task(jnp.minimum(t + 1, NT - 1), 16 * i, nxt_s)))
            at += 1.6
            for fn in work[9 * i:9 * i + 9]:
                tasks.append((at, int(at) + 3, fn))
                at += 0.36
        st = _Stream(j < 0, tasks)
        aop[t] = cur_s[...]
        for p in range(NP):
            m = []
            for n in range(7):
                m.append(st.dot(_bf(cur_s[n]), column_op(n, wqkv_v.at[p], sqkv.at[p])))
                if p == NP - 1:
                    cur_s[n] = st.after(nxt_s[n], m[n])
            store_qkv(p, pl.multiple_of(t * HM, HM), _combine(m))
        return carry
    jax.lax.fori_loop(0, NT - 2, phase1, 0)

    def phase2(t, carry):
        r0 = pl.multiple_of(t * TM, TM)
        held = {}

        def gather_heads(g, i, lo, s):
            def fn(gate):
                rows = pl.ds(pl.multiple_of(t * HM + (lo + s * QM + 16 * i) // 2, 8), 8)
                tiles = [_spread(gate(qkv_v[2 * g + (c % 4) // 2, c // 4, rows, (c % 2) * L:(c % 2 + 1) * L]), 8 * s + c)
                         for c in range(8)]
                held[g, i, s] = _butterfly(tiles, 4)
                return [held[g, i, s][-1]]
            return fn

        def gather_blocks(g, i, dst, c0):
            def fn(gate):
                for c in range(c0, c0 + 2):
                    tiles = _butterfly([gate(held[g, i, s][c]) if s == 0 else held[g, i, s][c] for s in range(4)], 16)
                    for k, v in enumerate(tiles):
                        out = _flip(v, 8 * k + c)
                        dst[8 * k + c, 16 * i:16 * i + 16, :] = _unpack_group(out)
                return [out]
            return fn

        def relayout(g, dst, i, lo):
            return [gather_heads(g, i, lo, s) for s in range(4)] + [gather_blocks(g, i, dst, c) for c in range(0, 8, 2)]

        def scores(i, d0, dn):
            def fn(gate):
                b0 = 16 * i
                logits = held.setdefault(("logits", i), [None] * WIN)
                for d in range(d0, d0 + dn):
                    q = gate(q_s[d, b0:b0 + 16, :])
                    for w in range(WIN):
                        k0 = HALO + b0 - DIL * w
                        term = q * k_s[d, k0:k0 + 16, :]
                        logits[w] = term if d == 0 else logits[w] + term
                return [logits[-1][-8:]]
            return fn

        def softmax(i):
            def fn(gate):
                logits = [l * SCALE for l in held["logits", i]]
                if i == 0:
                    pos = (r0 + QM * (jax.lax.broadcasted_iota(i32, (16, L), 1) >> 5)
                           + jax.lax.broadcasted_iota(i32, (16, L), 0))
                    logits = [jnp.where(pos >= DIL * w, l, -1e9) if w else l for w, l in enumerate(logits)]
                mx = functools.reduce(jnp.maximum, logits)
                es = [jnp.exp(l - mx) for l in logits]
                inv = 1.0 / functools.reduce(jnp.add, es)
                held["weights", i] = [e * inv for e in es]
                return [inv]
            return fn

        def values(i, d0, dn):
            def fn(gate):
                b0 = 16 * i
                ps = list(held["weights", i])
                ps[0] = gate(ps[0])
                for d in range(d0, d0 + dn):
                    acc = ps[0] * v_s[d, HALO + b0:HALO + b0 + 16, :]
                    for w in range(1, WIN):
                        k0 = HALO + b0 - DIL * w
                        acc = acc + ps[w] * v_s[d, k0:k0 + 16, :]
                    out = _pack_groups(acc)
                    att_s[d, _half(b0, 16), :] = out
                return [out]
            return fn

        def scatter_blocks(i, c0):
            def fn(gate):
                for c in range(c0, c0 + 2):
                    tiles = [_flip(gate(att_s[8 * k + c, _half(16 * i, 16), :]), 8 * k + c) for k in range(4)]
                    held["out", i, c] = _butterfly(tiles, 16)
                return [held["out", i, c][-1]]
            return fn

        def scatter_heads(i, s):
            def fn(gate):
                rows = []
                for s1 in (s, s + 2):
                    tiles = [held["out", i, c][s1] for c in range(8)]
                    tiles = _butterfly([gate(tiles[0])] + tiles[1:], 4)
                    rows.append([_unpack_group(_unspread(v, 8 * s1 + c)) for c, v in enumerate(tiles)])
                for c in range(0, 4, 2):
                    part = lambda k, c1: jnp.concatenate(rows[k][c1:c1 + 2], axis=1)
                    ops = _a_ops(part(0, c), part(0, c + 4), part(1, c), part(1, c + 4))
                    for n, v in enumerate(ops):
                        a_s[n, s * QM + 16 * i:s * QM + 16 * i + 16, c * L:(c + 2) * L] = v.astype(bf16)
                return [ops[0][-8:, -L:]]
            return fn

        tasks = []
        at = -0.2

        def place(fns, span, slack=4):
            nonlocal at
            for fn in fns:
                tasks.append((at, int(at + span) + slack, fn))
                at += span

        for i in range(4):
            place(relayout(0, q_s, i, HALO), 0.2)
            if i == 0:
                place(relayout(1, k_s, 0, 0), 0.2)
            place(relayout(1, k_s, i + 1, 0), 0.2)
            place([scores(i, d, 4) for d in range(0, DH, 4)], 0.9)
            place([softmax(i)], 0.3)
            if i == 0:
                place(relayout(2, v_s, 0, 0), 0.2)
            place(relayout(2, v_s, i + 1, 0), 0.2)
            place([values(i, d, 4) for d in range(0, DH, 4)], 0.9)
            place([scatter_blocks(i, c) for c in range(0, 8, 2)], 0.2)
            place([scatter_heads(i, s) for s in range(2)], 0.8)
        assert at < 14 * NC - 1, at
        st = _Stream(t < 0, tasks)

        for c in range(NC):
            gu = []
            for q in (c, NC + c):
                gu.append(_combine([st.dot(_bf(aop[t, n]), column_op(n, wc_v.at[q], sc.at[q])) for n in range(7)]))
            h = [jax.nn.gelu(g, approximate=True) * u for g, u in zip(*gu)]
            for n, v in enumerate(_a_ops(*h)):
                h_s[n, :, c * CW:(c + 1) * CW] = v.astype(bf16)

        m = [st.dot(a_s[n], jnp.concatenate([column_op(n, wc_v.at[q], sc.at[q]) for q in range(2 * NC, NQ)], axis=1))
             for n in range(7)]
        for n in range(7):
            m[n] = m[n] + st.dot(h_s[n], right_op(
                n, lambda i: sd[i].reshape(F2 // 2, D2),
                lambda: wd_v[0, :, :, :D2].reshape(F2, D2), lambda: wd_v[1, :, :, D2:].reshape(F2, D2)))
        c11, c12, c21, c22 = _combine(m)
        for block, r, c in ((c21, HM, 0), (c12, 0, D2), (c22, HM, D2), (c11, 0, 0)):
            at = (pl.ds(r0 + r, HM), pl.ds(c, D2))
            o_v[at] = (block + x_v[at].astype(f32)).astype(bf16)
            pltpu.make_async_copy(o_v.at[at], o_hbm.at[at], sem_o).start()
        return carry
    jax.lax.fori_loop(0, NT, phase2, 0)
    pltpu.make_async_copy(o_v, o_hbm, sem_o).wait()


@jax.jit
def pallas_parallel_sum__sliding_local_dilated__glu_gated_geglu__prompt_kernel(A_x, A_wqkv, A_wo, B_x, B_w_gate, B_w_up, B_w_down):
    x = A_x.reshape(S, D)
    V = pltpu.VMEM
    DMA = pltpu.SemaphoreType.DMA
    out = pl.pallas_call(
        _kernel,
        in_specs=[pl.BlockSpec(memory_space=pl.ANY)] * 6,
        out_specs=pl.BlockSpec(memory_space=pl.ANY),
        out_shape=jax.ShapeDtypeStruct((S, D), A_x.dtype),
        scratch_shapes=[
            V((S, D), bf16), V((NP, 2, D, CW), bf16), V((NQ, 2, D, CW), bf16), V((2, NR, RW, D), bf16),
            V((NP, 5, D2 // 2, CW), i32), V((NQ, 5, D2 // 2, CW), i32), V((5, NR, RW // 2, D2), i32),
            V((NT, 7, HM // 2, D2), i32), V((NP, 2, (S + HALO) // 2, CW), i32),
            V((DH, QM, L), f32), V((DH, QM + HALO, L), f32), V((DH, QM + HALO, L), f32),
            V((DH, QM // 2, L), i32), V((7, HM // 2, D2), i32), V((7, HM // 2, D2), i32),
            V((7, HM, D2), bf16), V((7, HM, F2), bf16), V((S, D), bf16),
            DMA((NT,)), DMA((NP,)), DMA((NQ,)), DMA((NR,)), DMA(()),
        ],
        compiler_params=pltpu.CompilerParams(vmem_limit_bytes=120 * 1024 * 1024),
    )(x, A_wqkv, A_wo, B_w_gate, B_w_up, B_w_down)
    return out.reshape(A_x.shape)
```

```python
import functools

import jax
import jax.experimental.pallas as pl
import jax.experimental.pallas.tpu as pltpu
import jax.numpy as jnp
import numpy as np

S, D, F = 2048, 1024, 3584
DH = 32
WIN, DIL = 8, 2
LN_EPS = 1e-5
SCALE = DH ** -0.5

L = 128
HALO = 16
TM = 256
HM, QM = TM // 2, TM // 4
NT = S // TM
D2, F2 = D // 2, F // 2
CW = 256
RW = 128
NP = 3 * D2 // CW
NC = F2 // CW
NQ = 2 * NC + D2 // CW
NR = F2 // RW

bf16, f32, i32 = jnp.bfloat16, jnp.float32, jnp.int32


def _half(r, n):
    return slice(r // 2, (r + n) // 2)


def _pack(v):
    return pltpu.bitcast(v.astype(bf16), i32)


def _bf(words):
    return pltpu.bitcast(words, bf16)


def _pack_groups(v):
    lo, hi = ([v[r:r + 8] for r in range(k, v.shape[0], 16)] for k in (0, 8))
    return pltpu.pack_elementwise([jnp.concatenate(lo, axis=0), jnp.concatenate(hi, axis=0)], packed_dtype=bf16)


def _unpack_group(words):
    return jnp.concatenate(
        [pltpu.unpack_elementwise(words, index=k, packed_dtype=bf16, unpacked_dtype=f32) for k in range(2)], axis=0)


def _lane(tile):
    return jax.lax.broadcasted_iota(i32, tile.shape, 1)


def _spread(tile, m):
    lane = _lane(tile)
    return jnp.take_along_axis(tile, (lane & 3) * 32 + ((lane >> 2) ^ m), axis=1)


def _unspread(tile, m):
    lane = _lane(tile)
    return jnp.take_along_axis(tile, ((lane & 31) ^ m) * 4 + (lane >> 5), axis=1)


def _flip(tile, m):
    return jnp.take_along_axis(tile, _lane(tile) ^ (4 * m), axis=1) if m else tile


def _butterfly(tiles, bit):
    n = len(tiles) // 2
    if n == 0:
        return tiles
    take = ((_lane(tiles[0]) >> 2) & bit) != 0
    lo = [jnp.where(take, b, a) for a, b in zip(tiles[:n], tiles[n:])]
    hi = [jnp.where(take, a, b) for a, b in zip(tiles[:n], tiles[n:])]
    return _butterfly(lo, bit // 2) + _butterfly(hi, bit // 2)


def _left_ops(a11, a12, a21, a22):
    return [a11 + a22, a21 + a22, a11, a22, a11 + a12, a21 - a11, a12 - a22]


def _right_sums(b11, b12, b21, b22):
    return [b11 + b22, b12 - b22, b21 - b11, b11 + b12, b21 + b22]


def _right_op(n, sums, b11, b22):
    return b11() if n == 1 else b22() if n == 4 else _bf(sums((0, None, 1, 2, None, 3, 4)[n]))


def _combine(m):
    return m[0] + m[3] - m[4] + m[6], m[2] + m[4], m[1] + m[3], m[0] - m[1] + m[2] + m[5]


def _geglu(g, u):
    c = float(np.sqrt(2.0 / np.pi))
    th = jnp.tanh(g * (c + (0.044715 * c) * (g * g)))
    half = (0.5 * g) * u
    return half * th + half


class _Stream:
    def __init__(self, never, tasks):
        self.never = never
        self.tasks = tasks
        self.count = 0
        self.due = {}

    def _tie(self, v, token):
        w = pltpu.bitcast(v, i32)
        t = jnp.concatenate([token] * (w.shape[0] // 8), axis=0)
        t = jnp.concatenate([t] * (w.shape[1] // L), axis=1)
        return pltpu.bitcast(jnp.where(self.never, t, w), v.dtype)

    def after(self, v, result):
        return self._tie(v, pltpu.bitcast(result[:8, :L], i32))

    def _run(self, result):
        for start, finish, fn in self.tasks:
            if result is None and start < 0:
                gate = lambda v: v
            elif result is not None and self.count <= start < self.count + 1:
                rows, cols = result.shape[0] // 8, result.shape[1] // L
                at = int((start - self.count) * rows * cols)
                r, c = at % rows * 8, at // rows * L
                gate = functools.partial(self._tie, token=pltpu.bitcast(result[r:r + 8, c:c + L], i32))
            else:
                continue
            last = pltpu.bitcast(fn(gate), i32)
            for r in range(0, last.shape[0], 8):
                for c in range(0, last.shape[1], L):
                    piece = last[r:r + 8, c:c + L]
                    self.due[finish] = self.due[finish] | piece if finish in self.due else piece

    def dot(self, a, b):
        if self.count == 0:
            self._run(None)
        if self.count in self.due:
            a = jnp.concatenate([self._tie(a[:16], self.due.pop(self.count)), a[16:]], axis=0)
        result = jnp.dot(a, b, preferred_element_type=f32)
        self._run(result)
        self.count += 1
        return result


def _kernel(x_hbm, wqkv_hbm, wo_hbm, wg_hbm, wu_hbm, wd_hbm, o_hbm,
            x_v, wqkv_v, wc_v, wd_v, sqkv, sc, sd,
            aop, qkv_v, q_s, k_s, v_s, att_s, cur_s, nxt_s, a_s, h_s, o_v,
            sem_x, sem_qkv, sem_c, sem_d, sem_o):

    def x_copy(t):
        rows = pl.ds(pl.multiple_of(t * TM, TM), TM)
        return pltpu.make_async_copy(x_hbm.at[rows], x_v.at[rows], sem_x.at[t])

    def qkv_start(p):
        c0 = (p // 2) * D + (p % 2) * CW
        for h in range(2):
            pltpu.make_async_copy(wqkv_hbm.at[:, pl.ds(c0 + h * D2, CW)], wqkv_v.at[p, h], sem_qkv.at[p]).start()

    def weights_start(j):
        for q in range(3 * j, min(3 * j + 6, NQ)):
            w_hbm, c = (wg_hbm, wu_hbm, wo_hbm)[q // NC], q % NC
            for h in range(2):
                cols = pl.ds(h * (w_hbm.shape[1] // 2) + c * CW, CW)
                pltpu.make_async_copy(w_hbm.at[:, cols], wc_v.at[q, h], sem_c.at[q]).start()
        for e in range(3 * j, min(3 * j + 6, NR)):
            for h in range(2):
                pltpu.make_async_copy(wd_hbm.at[pl.ds(h * F2 + e * RW, RW)], wd_v.at[h, e], sem_d.at[e]).start()

    def filled(buf, sem):
        pltpu.make_async_copy(buf, buf, sem).wait()

    def layernorm(r0, gate):
        x = gate(x_v[pl.ds(pl.multiple_of(r0, 16), 16), :].astype(f32))
        xc = x - jnp.mean(x, axis=-1, keepdims=True)
        var = jnp.mean(xc * xc, axis=-1, keepdims=True)
        return xc * jax.lax.rsqrt(var + LN_EPS)

    def ln_task(t, r, dst):
        def fn(gate):
            top, bot = layernorm(t * TM + r, gate), layernorm(t * TM + HM + r, gate)
            ops = [_pack(v) for v in _left_ops(top[:, :D2], top[:, D2:], bot[:, :D2], bot[:, D2:])]
            for n, v in enumerate(ops):
                dst[n, pl.ds(pl.multiple_of(r // 2, 8), 8), :] = v
            return ops[0][:, -L:]
        return fn

    def sums_task(blocks, dst, r, n):
        def fn(gate):
            b11, b12, b21, b22 = (b.astype(f32) for b in blocks(r, n))
            sums = [_pack(v) for v in _right_sums(gate(b11), b12, b21, b22)]
            for i, v in enumerate(sums):
                dst(i)[_half(r, n), :] = v
            return sums[-1][-8:, -L:]
        return fn

    def column_tasks(w, s, n):
        blocks = lambda r, n: (w[0, r:r + n], w[1, r:r + n], w[0, D2 + r:D2 + r + n], w[1, D2 + r:D2 + r + n])
        return [sums_task(blocks, lambda i: s.at[i], r, n) for r in range(0, D2, n)]

    def row_tasks(e, n):
        blocks = lambda r, n: (wd_v[0, e, r:r + n, :D2], wd_v[0, e, r:r + n, D2:],
                               wd_v[1, e, r:r + n, :D2], wd_v[1, e, r:r + n, D2:])
        return [sums_task(blocks, lambda i: sd.at[i, e], r, n) for r in range(0, RW, n)]

    def column_op(n, w, s):
        return _right_op(n, lambda i: s[i], lambda: w[0, :D2], lambda: w[1, D2:])

    def store_qkv(p, r0, blocks):
        c11, c12, c21, c22 = blocks
        top, bot = pl.ds(r0 + HALO // 2, HM // 2), pl.ds(r0 + (HALO + HM) // 2, HM // 2)
        qkv_v[p, 0, bot, :] = _pack_groups(c21)
        qkv_v[p, 1, top, :] = _pack_groups(c12)
        qkv_v[p, 1, bot, :] = _pack_groups(c22)
        qkv_v[p, 0, top, :] = _pack_groups(c11)

    x_copy(0).start()
    x_copy(1).start()
    qkv_start(0)
    x_copy(0).wait()
    x_copy(2).start()
    for p in range(1, NP):
        qkv_start(p)
    for r in range(0, HM, 16):
        ln_task(0, r, aop.at[0])(lambda v: v)
    x_copy(1).wait()
    x_copy(3).start()
    weights_start(0)
    for r in range(0, HM, 16):
        ln_task(1, r, aop.at[1])(lambda v: v)

    def first_tiles(p, carry):
        filled(wqkv_v.at[p], sem_qkv.at[p])
        pl.when(p == 1)(lambda: x_copy(2).wait())
        for j in (2, 4):
            @pl.when(p == j - 2)
            def _():
                x_copy(j + 2).start()
                x_copy(j + 3).start()

            pl.when(p == j - 1)(functools.partial(weights_start, j))

        src, r0 = jnp.where(p == 0, 1, 2), jnp.clip(p - 1, 0, 3) * 32
        tasks = [((i - 1) * 0.055, 2, fn) for i, fn in enumerate(column_tasks(wqkv_v.at[p], sqkv.at[p], 16))]
        tasks += [(2.2 + 2.2 * i, 6 + i, ln_task(src, r0 + 16 * i, cur_s)) for i in range(2)]
        stream = _Stream(p < 0, tasks)
        m = [None] * 7
        for n in (1, 4, 0, 2, 3, 5, 6):
            a = jnp.concatenate([aop[0, n], aop[1, n]], axis=0)
            m[n] = stream.dot(_bf(a), column_op(n, wqkv_v.at[p], sqkv.at[p]))
        for t in range(2):
            blocks = _combine([v[t * HM:(t + 1) * HM] for v in m])
            store_qkv(p, t * HM, blocks)
            if t == 0:
                for h in range(2):
                    qkv_v[p, h, :HALO // 2, :] = _pack_groups(jnp.broadcast_to(blocks[h][0:1], (HALO, CW)))
        return carry

    jax.lax.fori_loop(0, NP, first_tiles, 0)

    def other_tiles(j, carry):
        t = j + 2
        for i in range(3):
            pl.when(3 * j + i < NQ)(lambda: filled(wc_v.at[3 * j + i], sem_c.at[3 * j + i]))
        for i in range(3):
            pl.when(3 * j + i < NR)(lambda: filled(wd_v.at[:, 3 * j + i], sem_d.at[3 * j + i]))
        pl.when(t + 1 < NT)(lambda: x_copy(t + 1).wait())

        work = []
        for i in range(3):
            q = jnp.minimum(3 * j + i, NQ - 1)
            work += column_tasks(wc_v.at[q], sc.at[q], 32) + row_tasks(jnp.minimum(3 * j + i, NR - 1), 16)
        tasks, at = [], -0.3
        for i in range(8):
            tasks.append((at, int(at) + 7, ln_task(jnp.minimum(t + 1, NT - 1), 16 * i, nxt_s)))
            at += 1.6
            for fn in work[9 * i:9 * i + 9]:
                tasks.append((at, int(at) + 5, fn))
                at += 0.36
        stream = _Stream(j < 0, tasks)
        aop[t] = cur_s[...]
        for p in range(NP):
            m = []
            for n in range(7):
                m.append(stream.dot(_bf(cur_s[n]), column_op(n, wqkv_v.at[p], sqkv.at[p])))
                if p == NP - 1:
                    cur_s[n] = stream.after(nxt_s[n], m[n])
            store_qkv(p, pl.multiple_of(t * HM, HM), _combine(m))
        return carry

    jax.lax.fori_loop(0, NT - 2, other_tiles, 0)

    def output_tile(t, carry):
        r0 = pl.multiple_of(t * TM, TM)
        held = {}

        def gather_heads(g, i, lo, s):
            def fn(gate):
                rows = pl.ds(pl.multiple_of(t * HM + (lo + s * QM + 16 * i) // 2, 8), 8)
                tiles = [_spread(gate(qkv_v[2 * g + (c % 4) // 2, c // 4, rows, (c % 2) * L:(c % 2 + 1) * L]), 8 * s + c)
                         for c in range(8)]
                held[g, i, s] = _butterfly(tiles, 4)
                return held[g, i, s][-1]
            return fn

        def gather_blocks(g, i, dst, c0):
            def fn(gate):
                for c in range(c0, c0 + 2):
                    tiles = _butterfly([gate(held[g, i, 0][c])] + [held[g, i, s][c] for s in range(1, 4)], 16)
                    for k, v in enumerate(tiles):
                        out = _flip(v, 8 * k + c)
                        dst[8 * k + c, 16 * i:16 * i + 16, :] = _unpack_group(out)
                return out
            return fn

        def relayout(g, dst, i, lo):
            return [gather_heads(g, i, lo, s) for s in range(4)] + [gather_blocks(g, i, dst, c) for c in range(0, 8, 2)]

        def shifted(src, d, i, w):
            r = HALO + 16 * i - DIL * w
            return src[d, r:r + 16, :]

        def scores(i, d0, dn):
            def fn(gate):
                logits = held.setdefault(("logits", i), [None] * WIN)
                for d in range(d0, d0 + dn):
                    q = gate(q_s[d, 16 * i:16 * i + 16, :])
                    for w in range(WIN):
                        term = q * shifted(k_s, d, i, w)
                        logits[w] = term if d == 0 else logits[w] + term
                return logits[-1][-8:]
            return fn

        def softmax(i):
            def fn(gate):
                logits = [v * SCALE for v in held["logits", i]]
                if i == 0:
                    pos = r0 + QM * (_lane(logits[0]) >> 5) + jax.lax.broadcasted_iota(i32, (16, L), 0)
                    logits = [jnp.where(pos >= DIL * w, v, -1e9) if w else v for w, v in enumerate(logits)]
                top = functools.reduce(jnp.maximum, logits)
                es = [jnp.exp(v - top) for v in logits]
                inv = 1.0 / functools.reduce(jnp.add, es)
                held["weights", i] = [e * inv for e in es]
                return inv
            return fn

        def values(i, d):
            def fn(gate):
                weights = held["weights", i]
                acc = gate(weights[0]) * shifted(v_s, d, i, 0)
                for w in range(1, WIN):
                    acc = acc + weights[w] * shifted(v_s, d, i, w)
                out = _pack_groups(acc)
                att_s[d, _half(16 * i, 16), :] = out
                return out
            return fn

        def scatter_blocks(i, c0):
            def fn(gate):
                for c in range(c0, c0 + 2):
                    tiles = [_flip(gate(att_s[8 * k + c, _half(16 * i, 16), :]), 8 * k + c) for k in range(4)]
                    held["out", i, c] = _butterfly(tiles, 16)
                return held["out", i, c][-1]
            return fn

        def scatter_heads(i, s):
            def fn(gate):
                rows = []
                for s1 in (s, s + 2):
                    tiles = [held["out", i, c][s1] for c in range(8)]
                    tiles = _butterfly([gate(tiles[0])] + tiles[1:], 4)
                    rows.append([_unpack_group(_unspread(v, 8 * s1 + c)) for c, v in enumerate(tiles)])
                part = lambda k, c: jnp.concatenate(rows[k][c:c + 2], axis=1)
                for c in range(0, 4, 2):
                    ops = _left_ops(part(0, c), part(0, c + 4), part(1, c), part(1, c + 4))
                    for n, v in enumerate(ops):
                        a_s[n, s * QM + 16 * i:s * QM + 16 * i + 16, c * L:(c + 2) * L] = v.astype(bf16)
                return ops[0][-8:, -L:]
            return fn

        tasks, at = [], -0.2

        def place(fns, span):
            nonlocal at
            for fn in fns:
                tasks.append((at, int(at + span) + 6, fn))
                at += span

        for i in range(QM // 16):
            place(relayout(0, q_s, i, HALO), 0.22)
            for i1 in range(i + 1 if i else 0, i + 2):
                place(relayout(1, k_s, i1, 0), 0.22)
            place([scores(i, d, 2) for d in range(0, DH, 2)], 0.41)
            place([softmax(i)], 0.2)
            for i1 in range(i + 1 if i else 0, i + 2):
                place(relayout(2, v_s, i1, 0), 0.22)
            place([values(i, d) for d in range(DH)], 0.205)
            place([scatter_blocks(i, c) for c in range(0, 8, 2)], 0.25)
            place([scatter_heads(i, s) for s in range(2)], 1.0)
        assert at < 14 * NC
        stream = _Stream(t < 0, tasks)

        for c in range(NC):
            gate_up = [_combine([stream.dot(_bf(aop[t, n]), column_op(n, wc_v.at[q], sc.at[q])) for n in range(7)])
                       for q in (c, NC + c)]
            for n, v in enumerate(_left_ops(*(_geglu(g, u) for g, u in zip(*gate_up)))):
                h_s[n, :, c * CW:(c + 1) * CW] = v.astype(bf16)

        m = [stream.dot(a_s[n], jnp.concatenate(
            [column_op(n, wc_v.at[q], sc.at[q]) for q in range(2 * NC, NQ)], axis=1)) for n in range(7)]
        for n in range(7):
            m[n] = m[n] + stream.dot(h_s[n], _right_op(
                n, lambda i: sd[i].reshape(F2 // 2, D2),
                lambda: wd_v[0, :, :, :D2].reshape(F2, D2), lambda: wd_v[1, :, :, D2:].reshape(F2, D2)))
        c11, c12, c21, c22 = _combine(m)
        for block, r, c in ((c21, HM, 0), (c12, 0, D2), (c22, HM, D2), (c11, 0, 0)):
            at_rc = (pl.ds(r0 + r, HM), pl.ds(c, D2))
            o_v[at_rc] = (block + x_v[at_rc].astype(f32)).astype(o_v.dtype)
            pltpu.make_async_copy(o_v.at[at_rc], o_hbm.at[at_rc], sem_o).start()
        return carry

    jax.lax.fori_loop(0, NT, output_tile, 0)
    pltpu.make_async_copy(o_v, o_hbm, sem_o).wait()


@jax.jit
def pallas_parallel_sum__sliding_local_dilated__glu_gated_geglu__prompt_kernel(
    A_x: jax.Array,
    A_wqkv: jax.Array,
    A_wo: jax.Array,
    B_x: jax.Array,
    B_w_gate: jax.Array,
    B_w_up: jax.Array,
    B_w_down: jax.Array,
):
    del B_x
    vmem, dma = pltpu.VMEM, pltpu.SemaphoreType.DMA
    out = pl.pallas_call(
        _kernel,
        in_specs=[pl.BlockSpec(memory_space=pl.ANY)] * 6,
        out_specs=pl.BlockSpec(memory_space=pl.ANY),
        out_shape=jax.ShapeDtypeStruct((S, D), A_x.dtype),
        scratch_shapes=[
            vmem((S, D), bf16),
            vmem((NP, 2, D, CW), bf16),
            vmem((NQ, 2, D, CW), bf16),
            vmem((2, NR, RW, D), bf16),
            vmem((NP, 5, D2 // 2, CW), i32),
            vmem((NQ, 5, D2 // 2, CW), i32),
            vmem((5, NR, RW // 2, D2), i32),
            vmem((NT, 7, HM // 2, D2), i32),
            vmem((NP, 2, (HALO + S) // 2, CW), i32),
            vmem((DH, QM, L), f32),
            vmem((DH, HALO + QM, L), f32),
            vmem((DH, HALO + QM, L), f32),
            vmem((DH, QM // 2, L), i32),
            vmem((7, HM // 2, D2), i32),
            vmem((7, HM // 2, D2), i32),
            vmem((7, HM, D2), bf16),
            vmem((7, HM, F2), bf16),
            vmem((S, D), A_x.dtype),
            dma((NT,)), dma((NP,)), dma((NQ,)), dma((NR,)), dma(()),
        ],
        compiler_params=pltpu.CompilerParams(vmem_limit_bytes=120 * 1024 * 1024),
    )(A_x.reshape(S, D), A_wqkv, A_wo, B_w_gate, B_w_up, B_w_down)
    return out.reshape(A_x.shape)
```
